```python
import jax
import jax.numpy as jnp

def _softmax(x, axis=-1):
    return jax.nn.softmax(x, axis=axis)
def _gelu(x):
    return jax.nn.gelu(x, approximate=True)
def _silu(x):
    return jax.nn.silu(x)
def _sigmoid(x):
    return jax.nn.sigmoid(x)
def _layernorm(x, axis=-1, eps=1e-5):
    m = jnp.mean(x, axis=axis, keepdims=True)
    v = jnp.var(x, axis=axis, keepdims=True)
    return (x - m) / jnp.sqrt(v + eps)
def _scatter_add(tgt, idx, src, axis=0):
    return tgt.at[idx].add(src)
def _segment_sum(src, seg, n):
    return jax.ops.segment_sum(src, seg, n)
class _Rng:
    def __init__(self, key):
        self._k = key
    def _next(self):
        self._k, sub = jax.random.split(self._k)
        return sub
    def normal(self, shape):
        return jax.random.normal(self._next(), shape, dtype=jnp.bfloat16)
    def randint(self, lo, hi, shape):
        return jax.random.randint(self._next(), shape, lo, hi, dtype=jnp.int32)
    def uniform(self, shape, lo=0.0, hi=1.0):
        return jax.random.uniform(self._next(), shape, jnp.bfloat16, lo, hi)
    def permutation(self, n):
        return jax.random.permutation(self._next(), n)


kernel_name = 'standalone__dcn_v2_cross__recsys'

def setup_inputs():
    _rng = _Rng(jax.random.key(int.from_bytes(__import__("os").urandom(4), "little")))
    _w = (lambda a: (lambda t: t.astype(jnp.bfloat16) if jnp.issubdtype(t.dtype, jnp.floating) else t)(jnp.asarray(a)))
    B, F, D, L = 16384, 26, 128, 6
    Din = min(F * D, 1024)
    return {
        "x0": _w((lambda *s: _rng.normal(s) * 0.05)(B, Din)),
        "ws": _w((lambda *s: _rng.normal(s) * 0.05)(L, Din, Din)),
        "bs": _w((lambda *s: _rng.normal(s) * 0.05)(L, Din)),
    }

def reference(x0, ws, bs):
    x = x0
    for l in range(ws.shape[0]):
        x = x0 * (x @ ws[l] + bs[l]) + x
    return x
```

```python
import jax
import jax.numpy as jnp
from jax.experimental import pallas as pl
from jax.experimental.pallas import tpu as pltpu


def _cross_kernel(x0_ref, w_ref, b_ref, o_ref):
    num_layers = w_ref.shape[0]
    x0 = x0_ref[...].astype(jnp.float32)
    x = x0
    xb = x0_ref[...]
    for l in range(num_layers):
        y = jnp.dot(xb, w_ref[l], preferred_element_type=jnp.float32)
        x = x0 * (y + b_ref[l].astype(jnp.float32)) + x
        xb = x.astype(jnp.bfloat16)
    o_ref[...] = xb


@jax.jit
def pallas_standalone__dcn_v2_cross__recsys_kernel(x0, ws, bs):
    B, D = x0.shape
    L = ws.shape[0]
    bm = 512
    return pl.pallas_call(
        _cross_kernel,
        grid=(B // bm,),
        in_specs=[
            pl.BlockSpec((bm, D), lambda i: (i, 0)),
            pl.BlockSpec((L, D, D), lambda i: (0, 0, 0), pipeline_mode=pl.Buffered(1)),
            pl.BlockSpec((L, 1, D), lambda i: (0, 0, 0), pipeline_mode=pl.Buffered(1)),
        ],
        out_specs=pl.BlockSpec((bm, D), lambda i: (i, 0)),
        out_shape=jax.ShapeDtypeStruct((B, D), x0.dtype),
        compiler_params=pltpu.CompilerParams(
            dimension_semantics=("parallel",),
            vmem_limit_bytes=100 * 1024 * 1024,
        ),
    )(x0, ws, bs.reshape(L, 1, D))
```

```python
import functools

import jax
import jax.numpy as jnp
from jax.experimental import pallas as pl
from jax.experimental.pallas import tpu as pltpu

_F32 = jnp.float32
_BF16 = jnp.bfloat16

_QUADS = [(0, 0), (0, 1), (1, 0), (1, 1)]
_ALG = [
    ([(1, (0, 0))], [(1, (0, 1)), (-1, (1, 1))], [(1, (0, 1)), (1, (1, 1))]),
    ([(1, (0, 0)), (1, (0, 1))], [(1, (1, 1))], [(1, (0, 1)), (-1, (0, 0))]),
    ([(1, (1, 0)), (1, (1, 1))], [(1, (0, 0))], [(1, (1, 0)), (-1, (1, 1))]),
    ([(1, (1, 1))], [(1, (1, 0)), (-1, (0, 0))], [(1, (1, 0)), (1, (0, 0))]),
    ([(1, (0, 0)), (1, (1, 1))], [(1, (0, 0)), (1, (1, 1))], [(1, (0, 0)), (1, (1, 1))]),
    ([(1, (0, 1)), (-1, (1, 1))], [(1, (1, 0)), (1, (1, 1))], [(1, (0, 0))]),
    ([(1, (1, 0)), (-1, (0, 0))], [(1, (0, 0)), (1, (0, 1))], [(1, (1, 1))]),
]
_LAST = {q: max(r for r in range(7) if any(t[1] == q for t in _ALG[r][2])) for q in _QUADS}


def _combine(terms, get):
    value = get(terms[0][1])
    for sign, q in terms[1:]:
        value = value + get(q) if sign == 1 else value - get(q)
    return value


def _accumulate(acc, key, sign, value):
    if key in acc:
        acc[key] = acc[key] + value if sign == 1 else acc[key] - value
    else:
        acc[key] = value if sign == 1 else -value


def _prepare_weights(w_ref, s_ref, l, rows=16, cols=128):
    n = s_ref.shape[-1]

    def body(t, carry):
        r0 = pl.multiple_of(t * rows, rows)
        for c0 in range(0, n, cols):
            w = {
                (qo, qi): w_ref[
                    l,
                    pl.ds((2 * qo[0] + qi[0]) * n + r0, rows),
                    pl.ds((2 * qo[1] + qi[1]) * n + c0, cols),
                ].astype(_F32)
                for qo in _QUADS
                for qi in _QUADS
            }
            for r in range(7):
                outer = {qi: _combine(_ALG[r][1], lambda qo: w[qo, qi]) for qi in _QUADS}
                for s in range(7):
                    s_ref[l, r * 7 + s, pl.ds(r0, rows), pl.ds(c0, cols)] = _combine(
                        _ALG[s][1], lambda qi: outer[qi]
                    ).astype(_BF16)
        return carry

    jax.lax.fori_loop(0, n // rows, body, 0)


def _cross_layer(x, x0, b_ref, s_ref, l):
    n = s_ref.shape[-1]
    y, x_next = {}, {}
    for r in range(7):
        c = {}
        for s in range(7):
            a = _combine(_ALG[r][0], lambda qo: _combine(_ALG[s][0], lambda qi: x[qo, qi]))
            p = jnp.dot(a.astype(_BF16), s_ref[l, r * 7 + s], preferred_element_type=_F32)
            for sign_i, qi in _ALG[s][2]:
                _accumulate(c, qi, sign_i, p)
                if _LAST[qi] != s:
                    continue
                for sign_o, qo in _ALG[r][2]:
                    _accumulate(y, (qo, qi), sign_o, c[qi])
                    if _LAST[qo] == r:
                        c0 = (2 * qo[1] + qi[1]) * n
                        b = b_ref[l : l + 1, c0 : c0 + n].astype(_F32)
                        x_next[qo, qi] = x0[qo, qi] * (y[qo, qi] + b) + x[qo, qi]
    return x_next


def _cross_kernel(x0_ref, w_hbm, b_ref, o_ref, w_ref, s_ref, sem):
    num_layers = w_ref.shape[0]
    h = x0_ref.shape[0] // 4
    n = s_ref.shape[-1]

    @pl.when(pl.program_id(0) == 0)
    def _():
        copy = lambda l: pltpu.make_async_copy(w_hbm.at[l], w_ref.at[l], sem.at[l])
        for l in range(num_layers):
            copy(l).start()

        def body(l, carry):
            copy(l).wait()
            _prepare_weights(w_ref, s_ref, l)
            return carry

        jax.lax.fori_loop(0, num_layers, body, 0)

    def block(qo, qi):
        r0, c0 = (2 * qo[0] + qi[0]) * h, (2 * qo[1] + qi[1]) * n
        return slice(r0, r0 + h), slice(c0, c0 + n)

    x0 = {(qo, qi): x0_ref[block(qo, qi)].astype(_F32) for qo in _QUADS for qi in _QUADS}
    x = x0
    for l in range(num_layers):
        x = _cross_layer(x, x0, b_ref, s_ref, l)
    for key, value in x.items():
        o_ref[block(*key)] = value.astype(o_ref.dtype)


@jax.jit
def pallas_standalone__dcn_v2_cross__recsys_kernel(x0, ws, bs):
    batch, d = x0.shape
    num_layers = ws.shape[0]
    bm = 512
    assert batch % bm == 0 and d % 512 == 0
    return pl.pallas_call(
        _cross_kernel,
        grid=(batch // bm,),
        in_specs=[
            pl.BlockSpec((bm, d), lambda i: (i, 0)),
            pl.BlockSpec(memory_space=pl.ANY),
            pl.BlockSpec((num_layers, d), lambda i: (0, 0), pipeline_mode=pl.Buffered(1)),
        ],
        out_specs=pl.BlockSpec((bm, d), lambda i: (i, 0)),
        out_shape=jax.ShapeDtypeStruct((batch, d), x0.dtype),
        scratch_shapes=[
            pltpu.VMEM((num_layers, d, d), _BF16),
            pltpu.VMEM((num_layers, 49, d // 4, d // 4), _BF16),
            pltpu.SemaphoreType.DMA((num_layers,)),
        ],
        compiler_params=pltpu.CompilerParams(
            dimension_semantics=("arbitrary",),
            vmem_limit_bytes=120 * 1024 * 1024,
        ),
    )(x0, ws, bs)
```

```python
import jax
import jax.numpy as jnp
from jax.experimental import pallas as pl
from jax.experimental.pallas import tpu as pltpu

_F32 = jnp.float32
_BF16 = jnp.bfloat16

_QUADS = [(0, 0), (0, 1), (1, 0), (1, 1)]
_ALG = [
    ([(1, (0, 0))], [(1, (0, 1)), (-1, (1, 1))], [(1, (0, 1)), (1, (1, 1))]),
    ([(1, (0, 0)), (1, (0, 1))], [(1, (1, 1))], [(1, (0, 1)), (-1, (0, 0))]),
    ([(1, (1, 0)), (1, (1, 1))], [(1, (0, 0))], [(1, (1, 0)), (-1, (1, 1))]),
    ([(1, (1, 1))], [(1, (1, 0)), (-1, (0, 0))], [(1, (1, 0)), (1, (0, 0))]),
    ([(1, (0, 0)), (1, (1, 1))], [(1, (0, 0)), (1, (1, 1))], [(1, (0, 0)), (1, (1, 1))]),
    ([(1, (0, 1)), (-1, (1, 1))], [(1, (1, 0)), (1, (1, 1))], [(1, (0, 0))]),
    ([(1, (1, 0)), (-1, (0, 0))], [(1, (0, 0)), (1, (0, 1))], [(1, (1, 1))]),
]
_OUTER = [0, 1, 3, 2, 6, 5, 4]
_INNER = [0, 1, 2, 3, 4, 5, 6]


def _last_writer(order):
    return {q: [r for r in order if any(t[1] == q for t in _ALG[r][2])][-1] for q in _QUADS}


_LAST_OUTER = _last_writer(_OUTER)
_LAST_INNER = _last_writer(_INNER)


def _combine(terms, get):
    value = get(terms[0][1])
    for sign, q in terms[1:]:
        value = value + get(q) if sign == 1 else value - get(q)
    return value


def _accumulate(acc, key, sign, value):
    if key in acc:
        acc[key] = acc[key] + value if sign == 1 else acc[key] - value
    else:
        acc[key] = value if sign == 1 else -value


def _prepare_weights(w_ref, s_ref, l, rows=16, cols=128):
    n = s_ref.shape[-1]

    def body(t, carry):
        r0 = pl.multiple_of(t * rows, rows)
        p0 = pl.multiple_of(t * (rows // 2), rows // 2)
        for c0 in range(0, n, cols):
            w = {
                (qo, qi): w_ref[
                    l,
                    pl.ds((2 * qo[0] + qi[0]) * n + r0, rows),
                    pl.ds((2 * qo[1] + qi[1]) * n + c0, cols),
                ].astype(_F32)
                for qo in _QUADS
                for qi in _QUADS
            }
            for r in range(7):
                outer = {qi: _combine(_ALG[r][1], lambda qo: w[qo, qi]) for qi in _QUADS}
                for s in range(7):
                    v = _combine(_ALG[s][1], lambda qi: outer[qi]).astype(_BF16)
                    s_ref[l, r * 7 + s, pl.ds(p0, rows // 2), pl.ds(c0, cols)] = (
                        pltpu.bitcast(v, jnp.int32)
                    )
        return carry

    jax.lax.fori_loop(0, n // rows, body, 0)


def _cross_layer(x, x0, b_ref, s_ref, l):
    n = s_ref.shape[-1]
    y, x_next = {}, {}
    for r in _OUTER:
        c = {}
        for s in _INNER:
            a = _combine(_ALG[r][0], lambda qo: _combine(_ALG[s][0], lambda qi: x[qo, qi]))
            w = pltpu.bitcast(s_ref[l, r * 7 + s], _BF16)
            p = jnp.dot(a.astype(_BF16), w, preferred_element_type=_F32)
            for sign_i, qi in _ALG[s][2]:
                _accumulate(c, qi, sign_i, p)
                if _LAST_INNER[qi] != s:
                    continue
                for sign_o, qo in _ALG[r][2]:
                    _accumulate(y, (qo, qi), sign_o, c[qi])
                    if _LAST_OUTER[qo] == r:
                        c0 = (2 * qo[1] + qi[1]) * n
                        b = b_ref[l : l + 1, c0 : c0 + n].astype(_F32)
                        x_next[qo, qi] = x0[qo, qi] * (y[qo, qi] + b) + x[qo, qi]
    return x_next


def _cross_kernel(x0_ref, w_hbm, b_ref, o_ref, w_ref, s_ref, sem):
    num_layers = w_ref.shape[0]
    h = x0_ref.shape[0] // 4
    n = s_ref.shape[-1]
    keys = [(qo, qi) for qo in _QUADS for qi in _QUADS]

    def block(qo, qi):
        r0, c0 = (2 * qo[0] + qi[0]) * h, (2 * qo[1] + qi[1]) * n
        return slice(r0, r0 + h), slice(c0, c0 + n)

    @pl.when(pl.program_id(0) == 0)
    def _():
        copy = lambda l: pltpu.make_async_copy(w_hbm.at[l], w_ref.at[l], sem.at[l])
        for l in range(num_layers):
            copy(l).start()

        def body(l, carry):
            copy(l).wait()
            _prepare_weights(w_ref, s_ref, l)
            return carry

        jax.lax.fori_loop(0, num_layers, body, 0)

    x0 = {key: x0_ref[block(*key)].astype(_F32) for key in keys}
    x = x0
    for l in range(num_layers):
        x = _cross_layer(x, x0, b_ref, s_ref, l)
    for key, value in x.items():
        o_ref[block(*key)] = value.astype(o_ref.dtype)


@jax.jit
def pallas_standalone__dcn_v2_cross__recsys_kernel(x0, ws, bs):
    batch, d = x0.shape
    num_layers = ws.shape[0]
    bm = 512
    assert batch % bm == 0 and d % 512 == 0
    return pl.pallas_call(
        _cross_kernel,
        grid=(batch // bm,),
        in_specs=[
            pl.BlockSpec((bm, d), lambda i: (i, 0)),
            pl.BlockSpec(memory_space=pl.ANY),
            pl.BlockSpec((num_layers, d), lambda i: (0, 0), pipeline_mode=pl.Buffered(1)),
        ],
        out_specs=pl.BlockSpec((bm, d), lambda i: (i, 0)),
        out_shape=jax.ShapeDtypeStruct((batch, d), x0.dtype),
        scratch_shapes=[
            pltpu.VMEM((num_layers, d, d), _BF16),
            pltpu.VMEM((num_layers, 49, d // 8, d // 4), jnp.int32),
            pltpu.SemaphoreType.DMA((num_layers,)),
        ],
        compiler_params=pltpu.CompilerParams(
            dimension_semantics=("arbitrary",),
            vmem_limit_bytes=120 * 1024 * 1024,
        ),
    )(x0, ws, bs)
```
